```python
import os as _os
_os.environ.setdefault("JAX_PLATFORMS", "cpu")
import jax
import jax.numpy as jnp

def _softmax(x, axis=-1):
    return jax.nn.softmax(x, axis=axis)
def _gelu(x):
    return jax.nn.gelu(x, approximate=True)
def _silu(x):
    return jax.nn.silu(x)
def _sigmoid(x):
    return jax.nn.sigmoid(x)
def _layernorm(x, axis=-1, eps=1e-5):
    m = jnp.mean(x, axis=axis, keepdims=True)
    v = jnp.var(x, axis=axis, keepdims=True)
    return (x - m) / jnp.sqrt(v + eps)
def _scatter_add(tgt, idx, src, axis=0):
    return tgt.at[idx].add(src)
def _segment_sum(src, seg, n):
    return jax.ops.segment_sum(src, seg, n)
class _Rng:
    def __init__(self, key):
        self._k = key
    def _next(self):
        self._k, sub = jax.random.split(self._k)
        return sub
    def normal(self, shape):
        return jax.random.normal(self._next(), shape, dtype=jnp.bfloat16)
    def randint(self, lo, hi, shape):
        return jax.random.randint(self._next(), shape, lo, hi, dtype=jnp.int32)
    def uniform(self, shape, lo=0.0, hi=1.0):
        return jax.random.uniform(self._next(), shape, jnp.bfloat16, lo, hi)
    def permutation(self, n):
        return jax.random.permutation(self._next(), n)


kernel_name = 'sequential_preLN__linear_attn_block__glu_gated_reglu__prompt'

def setup_inputs():
    _rng = _Rng(jax.random.key(int.from_bytes(__import__("os").urandom(4), "little")))
    _w = (lambda a: (lambda t: t.astype(jnp.bfloat16) if jnp.issubdtype(t.dtype, jnp.floating) else t)(jnp.asarray(a)))
    def _A_setup():
        B, S, D = 1, 2048, 640
        return {
            "x": _w((lambda *s: _rng.normal(s) * 0.05)(B, S, D)),
            "wqkv": _w((lambda *s: _rng.normal(s) * 0.05)(D, 3 * D)),
            "wo": _w((lambda *s: _rng.normal(s) * 0.05)(D, D)),
        }
    _A_in = _A_setup()

    def _B_setup():
        B, S, D, F = 1, 2048, 640, 1536
        return {
            "x": _w((lambda *s: _rng.normal(s) * 0.05)(B, S, D)),
            "W_gate": _w((lambda *s: _rng.normal(s) * 0.05)(D, F) * (2.0 / D) ** 0.5),
            "W_up": _w((lambda *s: _rng.normal(s) * 0.05)(D, F) * (2.0 / D) ** 0.5),
            "W_down": _w((lambda *s: _rng.normal(s) * 0.05)(F, D) * (1.0 / F) ** 0.5),
        }
    _B_in = _B_setup()

    return {
        "A_x": _A_in["x"],
        "A_wqkv": _A_in["wqkv"],
        "A_wo": _A_in["wo"],
        "B_x": _B_in["x"],
        "B_W_gate": _B_in["W_gate"],
        "B_W_up": _B_in["W_up"],
        "B_W_down": _B_in["W_down"],
    }

def reference(A_x, A_wqkv, A_wo, B_x, B_W_gate, B_W_up, B_W_down):
    def _A_ref(x, wqkv, wo):
        B, S, D = x.shape
        H = 32; Dh = D // H
        qkv = (lambda x, *d: x.transpose(*d))((x @ wqkv).reshape(B, S, 3, H, Dh), 2, 0, 3, 1, 4)
        q, k, v = qkv[0], qkv[1], qkv[2]
        phi = lambda t: jnp.where(t > 0, t + 1, jnp.exp(t)) + 1e-6
        pq, pk = phi(q), phi(k)
        kv = jnp.einsum("bhsd,bhse->bhde", pk, v)
        z = jnp.einsum("bhsd->bhd", pk)
        num = jnp.einsum("bhqd,bhde->bhqe", pq, kv)
        den = jnp.einsum("bhqd,bhd->bhq", pq, z)[..., None] + 1e-6
        o = num / den
        return (lambda x, *d: x.transpose(*d))(o, 0, 2, 1, 3).reshape(B, S, D) @ wo

    def _B_ref(x, W_gate, W_up, W_down):
        gate = jnp.einsum("bsd,df->bsf", x, W_gate)
        up = jnp.einsum("bsd,df->bsf", x, W_up)
        gate = gate * (lambda x, dt: x.astype(dt))(gate > 0, gate.dtype)
        h = gate * up
        return jnp.einsum("bsf,fd->bsd", h, W_down)

    x = A_x
    h = x + _A_ref(_layernorm(x, axis=-1), A_wqkv, A_wo)
    h2 = h + _B_ref(_layernorm(h, axis=-1), B_W_gate, B_W_up, B_W_down)
    return h2
```

```python
import functools
import jax
import jax.numpy as jnp
from jax import lax
import jax.experimental.pallas as pl
import jax.experimental.pallas.tpu as pltpu

S = 2048
D = 640
F = 1536
H = 32
DH = 20
TM = 256
NT = S // TM
NL = D // 128
ROWS = [(0, 144), (112, 272), (240, 400), (368, 528), (496, 640)]
EPS = 1e-5
LAST_SPLIT = [(0, 192), (192, 256)]
f32 = jnp.float32
bf16 = jnp.bfloat16


def _ln(x):
    m = jnp.mean(x, axis=-1, keepdims=True)
    xc = x - m
    v = jnp.mean(xc * xc, axis=-1, keepdims=True)
    return xc * lax.rsqrt(v + EPS)


def _phi(t):
    return jnp.where(t > 0, t + 1.0, jnp.exp(t)) + 1e-6


def _dot(a, b):
    return jnp.dot(a, b, preferred_element_type=f32)


def _dot_nt(a, b):
    return lax.dot_general(a, b, (((1,), (1,)), ((), ())), preferred_element_type=f32)


def _head(idx):
    return lax.shift_right_logical(idx * 3277, 16)


def _kernel(x_hbm, wqkv_hbm, wo_hbm, wg_hbm, wu_hbm, wd_hbm, out_hbm,
            x_v, xn_v, out_v, wq_v, wk_v, wv_v, wkT_v, wo_v, wg_v, wu_v, wd_v,
            kv_acc, z_acc, m_acc, m_v, wqT32, wqTp_v, zp_v, zrow_v, xa_v, xb_v, h_v, hn_v, va_v, vb_v, pk_v,
            sem_x, sem_o, sem_w):

    def x_copy(t):
        return pltpu.make_async_copy(x_hbm.at[pl.ds(t * TM, TM)], x_v.at[pl.ds(t * TM, TM)], sem_x.at[t])

    def o_copy(t):
        return pltpu.make_async_copy(out_v.at[pl.ds(t * TM, TM)], out_hbm.at[pl.ds(t * TM, TM)], sem_o.at[t])

    c_wq = pltpu.make_async_copy(wqkv_hbm.at[:, pl.ds(0, D)], wq_v, sem_w.at[0])
    c_wk = pltpu.make_async_copy(wqkv_hbm.at[:, pl.ds(D, D)], wk_v, sem_w.at[1])
    c_wo = pltpu.make_async_copy(wo_hbm, wo_v, sem_w.at[3])
    c_wg = pltpu.make_async_copy(wg_hbm, wg_v, sem_w.at[4])
    c_wu = pltpu.make_async_copy(wu_hbm, wu_v, sem_w.at[5])
    c_wd = pltpu.make_async_copy(wd_hbm, wd_v, sem_w.at[6])

    VA = 256
    c_wva = pltpu.make_async_copy(wqkv_hbm.at[:, pl.ds(2 * D, VA)], wv_v.at[:, pl.ds(0, VA)], sem_w.at[2])
    c_wvb = pltpu.make_async_copy(wqkv_hbm.at[:, pl.ds(2 * D + VA, D - VA)], wv_v.at[:, pl.ds(VA, D - VA)], sem_w.at[7])

    x_copy(0).start()
    x_copy(1).start()
    c_wva.start()
    c_wvb.start()
    c_wk.start()
    for t in range(2, NT):
        x_copy(t).start()
    c_wq.start()
    c_wo.start()
    c_wg.start()
    c_wu.start()
    c_wd.start()

    kv_acc[...] = jnp.zeros_like(kv_acc)
    z_acc[...] = jnp.zeros_like(z_acc)
    m_acc[...] = jnp.zeros_like(m_acc)

    def ln_tile(t, buf):
        r0 = pl.multiple_of(t * TM, TM)
        x = x_v[pl.ds(r0, TM), :].astype(f32)
        xn = _ln(x).astype(bf16)
        xn_v[pl.ds(r0, TM), :] = xn
        buf[...] = xn

    def kt_stage(buf):
        kT = _dot_nt(wkT_v[...], buf[...])
        pkT = _phi(kT)
        zs = pkT[:, 0:128]
        for c in range(1, TM // 128):
            zs = zs + pkT[:, c * 128:(c + 1) * 128]
        z_acc[...] += zs
        return pkT.astype(bf16)

    def v_stage(buf):
        return _dot(buf[...], wv_v[...]).astype(bf16)

    def kv_stage(pkT_b, v):
        for j in range(NL):
            a, b = ROWS[j]
            kv_acc[a:b, j * 128:(j + 1) * 128] += _dot(pkT_b[a:b, :], v[:, j * 128:(j + 1) * 128])

    x_copy(0).wait()
    ln_tile(0, xa_v)
    x_copy(1).wait()
    ln_tile(1, xb_v)
    c_wva.wait()
    va_v[:, 0:VA] = _dot(xa_v[...], wv_v[:, 0:VA]).astype(bf16)
    vb_v[:, 0:VA] = _dot(xb_v[...], wv_v[:, 0:VA]).astype(bf16)
    c_wvb.wait()
    va_v[:, VA:D] = _dot(xa_v[...], wv_v[:, VA:D]).astype(bf16)
    c_wk.wait()
    wkT_v[...] = wk_v[...].T
    vb_v[:, VA:D] = _dot(xb_v[...], wv_v[:, VA:D]).astype(bf16)
    pk0 = kt_stage(xa_v)
    x_copy(2).wait()
    kv_stage(pk0, va_v[...])
    ln_tile(2, xa_v)
    pk_v[...] = kt_stage(xb_v)

    def phase0(i, carry):
        x_copy(2 * i + 1).wait()
        x_copy(2 * i + 2).wait()
        kv_stage(pk_v[...], vb_v[...])
        ln_tile(2 * i + 1, xb_v)
        pkx = kt_stage(xa_v)
        vx = v_stage(xa_v)
        kv_stage(pkx, vx)
        ln_tile(2 * i + 2, xa_v)
        pk_v[...] = kt_stage(xb_v)
        vb_v[...] = v_stage(xb_v)
        return carry

    lax.fori_loop(1, NT // 2 - 1, phase0, 0)
    x_copy(NT - 1).wait()
    c_wo.wait()
    c_wq.wait()
    for n in range(NL):
        wqT32[n] = wq_v[n * 128:(n + 1) * 128, :].astype(f32).T
    for d in range(DH):
        for n in range(NL):
            wqTp_v[d * H:(d + 1) * H, n * 128:(n + 1) * 128] = wqT32[n, pl.ds(d, H, stride=DH), :].astype(bf16)
    kv_stage(pk_v[...], vb_v[...])
    ln_tile(NT - 1, xb_v)
    pkx = kt_stage(xa_v)
    vx = v_stage(xa_v)
    kv_stage(pkx, vx)
    pky = kt_stage(xb_v)
    vy = v_stage(xb_v)
    kv_stage(pky, vy)

    def q_stage(t):
        r0 = pl.multiple_of(t * TM, TM)
        xn = xn_v[pl.ds(r0, TM), :]
        return _phi(_dot_nt(xn, wqTp_v[...]))

    def den_stage(pq):
        t = pq * zrow_v[...]
        s = t[:, 0:128]
        for j in range(1, NL):
            s = s + t[:, j * 128:(j + 1) * 128]
        s = s + pltpu.roll(s, 64, 1)
        s = s + pltpu.roll(s, 32, 1)
        r = 1.0 / (s + 1e-6)
        return jnp.concatenate([pq[:, j * 128:(j + 1) * 128] * r for j in range(NL)], axis=1).astype(bf16)

    def attn_stage(t, pqn):
        r0 = pl.multiple_of(t * TM, TM)
        attn = _dot(pqn, m_v[...])
        h = x_v[pl.ds(r0, TM), :].astype(f32) + attn
        h_v[pl.ds(r0, TM), :] = h
        hn_v[...] = _ln(h).astype(bf16)

    def down_stage(t, hh):
        r0 = pl.multiple_of(t * TM, TM)
        out = h_v[pl.ds(r0, TM), :] + _dot(hh, wd_v[...])
        out_v[pl.ds(r0, TM), :] = out.astype(bf16)
        o_copy(t).start()

    pq0 = q_stage(0)
    for j in range(NL):
        a, b = ROWS[j]
        d_idx = a + lax.broadcasted_iota(jnp.int32, (b - a, 128), 0)
        e_idx = j * 128 + lax.broadcasted_iota(jnp.int32, (b - a, 128), 1)
        same = _head(d_idx) == _head(e_idx)
        kvj = jnp.where(same, kv_acc[a:b, j * 128:(j + 1) * 128], 0.0).astype(bf16)
        mj = _dot(kvj, wo_v[j * 128:(j + 1) * 128, :])
        for n in range(NL):
            m_acc[n, a:b, :] += mj[:, n * 128:(n + 1) * 128]
    for d in range(DH):
        for n in range(NL):
            m_v[d * H:(d + 1) * H, n * 128:(n + 1) * 128] = m_acc[n, pl.ds(d, H, stride=DH), :].astype(bf16)
        zp_v[d * H:(d + 1) * H, :] = z_acc[pl.ds(d, H, stride=DH), :]
    zrow_v[...] = jnp.sum(zp_v[...].T, axis=0, keepdims=True)

    attn_stage(0, den_stage(pq0))
    c_wg.wait()
    c_wu.wait()
    c_wd.wait()

    def phase1(t, carry):
        hn = hn_v[...]
        pq = q_stage(t + 1)
        gate = _dot(hn, wg_v[...])
        pqn = den_stage(pq)
        up = _dot(hn, wu_v[...])
        hh = (jnp.maximum(gate, 0.0) * up).astype(bf16)
        attn_stage(t + 1, pqn)
        down_stage(t, hh)
        return carry

    lax.fori_loop(0, NT - 1, phase1, 0)
    hn = hn_v[...]
    gate = _dot(hn, wg_v[...])
    up = _dot(hn, wu_v[...])
    hh = (jnp.maximum(gate, 0.0) * up).astype(bf16)
    base = (NT - 1) * TM
    last_copies = []
    for ci, (a, b) in enumerate(LAST_SPLIT):
        out = h_v[base + a:base + b, :] + _dot(hh[a:b, :], wd_v[...])
        out_v[base + a:base + b, :] = out.astype(bf16)
        cp = pltpu.make_async_copy(out_v.at[pl.ds(base + a, b - a)], out_hbm.at[pl.ds(base + a, b - a)], sem_o.at[NT - 1 + ci])
        cp.start()
        last_copies.append(cp)
    for t in range(NT - 1):
        o_copy(t).wait()
    for cp in last_copies:
        cp.wait()


@jax.jit
def pallas_sequential_preLN__linear_attn_block__glu_gated_reglu__prompt_kernel(
    A_x, A_wqkv, A_wo, B_x, B_W_gate, B_W_up, B_W_down):
    x2 = A_x.reshape(S, D)
    any_spec = pl.BlockSpec(memory_space=pl.ANY)
    out = pl.pallas_call(
        _kernel,
        out_shape=jax.ShapeDtypeStruct((S, D), bf16),
        in_specs=[any_spec] * 6,
        out_specs=any_spec,
        scratch_shapes=[
            pltpu.VMEM((S, D), bf16),
            pltpu.VMEM((S, D), bf16),
            pltpu.VMEM((S, D), bf16),
            pltpu.VMEM((D, D), bf16),
            pltpu.VMEM((D, D), bf16),
            pltpu.VMEM((D, D), bf16),
            pltpu.VMEM((D, D), bf16),
            pltpu.VMEM((D, D), bf16),
            pltpu.VMEM((D, F), bf16),
            pltpu.VMEM((D, F), bf16),
            pltpu.VMEM((F, D), bf16),
            pltpu.VMEM((D, D), f32),
            pltpu.VMEM((D, 128), f32),
            pltpu.VMEM((NL, D, 128), f32),
            pltpu.VMEM((D, D), bf16),
            pltpu.VMEM((NL, D, 128), f32),
            pltpu.VMEM((D, D), bf16),
            pltpu.VMEM((D, 128), f32),
            pltpu.VMEM((1, D), f32),
            pltpu.VMEM((TM, D), bf16),
            pltpu.VMEM((TM, D), bf16),
            pltpu.VMEM((S, D), f32),
            pltpu.VMEM((TM, D), bf16),
            pltpu.VMEM((TM, D), bf16),
            pltpu.VMEM((TM, D), bf16),
            pltpu.VMEM((D, TM), bf16),
            pltpu.SemaphoreType.DMA((NT,)),
            pltpu.SemaphoreType.DMA((NT + 3,)),
            pltpu.SemaphoreType.DMA((8,)),
        ],
        compiler_params=pltpu.CompilerParams(vmem_limit_bytes=100 * 1024 * 1024),
    )(x2, A_wqkv, A_wo, B_W_gate, B_W_up, B_W_down)
    return out.reshape(A_x.shape)
```

```python
import jax
import jax.numpy as jnp
from jax import lax
import jax.experimental.pallas as pl
import jax.experimental.pallas.tpu as pltpu

S = 2048
D = 640
F = 1536
H = 32
DH = 20
TM = 256
NT = S // TM
NL = D // 128
ROWS = [(0, 144), (112, 272), (240, 400), (368, 528), (496, 640)]
EPS = 1e-5
DP = D + 32
VCH = [(0, 128), (128, 640)]
V2 = 256
LAST_SPLIT = [(0, 192), (192, 256)]
f32 = jnp.float32
bf16 = jnp.bfloat16
u32 = jnp.uint32


def _ln(x):
    m = jnp.mean(x, axis=-1, keepdims=True)
    xc = x - m
    v = jnp.mean(xc * xc, axis=-1, keepdims=True)
    return xc * lax.rsqrt(v + EPS)


def _phi(t):
    return jnp.where(t > 0, t + 1.0, jnp.exp(t)) + 1e-6


def _dot(a, b):
    return jnp.dot(a, b, preferred_element_type=f32)


def _dot_nt(a, b):
    return lax.dot_general(a, b, (((1,), (1,)), ((), ())), preferred_element_type=f32)


def _head(idx):
    return lax.shift_right_logical(idx * 3277, 16)


def _pk(val):
    return pltpu.bitcast(val, u32)


def _up(val):
    return pltpu.bitcast(val, bf16)


def _kernel(x_hbm, wqkv_hbm, wo_hbm, wg_hbm, wu_hbm, wd_hbm, out_hbm,
            x_v, xn_v, out_v, wq_v, wk_v, wv_v, wkT_v, wo_v, wg_v, wu_v, wd_v,
            kv_acc, z_acc, m_acc, m_v, wqT32, wqTp_v, zp_v, xa_v, xb_v, h_v, hn_v,
            va_v, vb_v, pk_v, wvp_v, xc_v, vx_v, zrow_v,
            sem_x, sem_o, sem_w):

    def x_copy(t):
        return pltpu.make_async_copy(x_hbm.at[pl.ds(t * TM, TM)], x_v.at[pl.ds(t * TM, TM)], sem_x.at[t])

    def o_copy(t):
        return pltpu.make_async_copy(out_v.at[pl.ds(t * TM, TM)], out_hbm.at[pl.ds(t * TM, TM)], sem_o.at[t])

    c_wq = pltpu.make_async_copy(wqkv_hbm.at[:, pl.ds(0, D)], wq_v, sem_w.at[0])
    c_wk = pltpu.make_async_copy(wqkv_hbm.at[:, pl.ds(D, D)], wk_v, sem_w.at[1])
    c_wo = pltpu.make_async_copy(wo_hbm, wo_v, sem_w.at[3])
    c_wg = pltpu.make_async_copy(wg_hbm, wg_v, sem_w.at[4])
    c_wu = pltpu.make_async_copy(wu_hbm, wu_v, sem_w.at[5])
    c_wd = pltpu.make_async_copy(wd_hbm, wd_v, sem_w.at[6])
    c_wv = [pltpu.make_async_copy(wqkv_hbm.at[:, pl.ds(2 * D + s, e - s)], wv_v.at[:, pl.ds(s, e - s)],
                                  sem_w.at[7 + i]) for i, (s, e) in enumerate(VCH)]

    x_copy(0).start()
    x_copy(1).start()
    for c in c_wv:
        c.start()
    x_copy(2).start()
    c_wk.start()
    for t in range(3, NT):
        x_copy(t).start()
    c_wq.start()
    c_wo.start()
    c_wg.start()
    c_wu.start()
    c_wd.start()

    kv_acc[...] = jnp.zeros_like(kv_acc)
    z_acc[0:D, :] = jnp.zeros((D, 128), f32)
    m_acc[:, 0:D, :] = jnp.zeros((NL, D, 128), f32)

    def ln_tile(t, buf):
        r0 = pl.multiple_of(t * TM, TM)
        p0 = pl.multiple_of(t * (TM // 2), TM // 2)
        x = x_v[pl.ds(r0, TM), :].astype(f32)
        xn = _pk(_ln(x).astype(bf16))
        xn_v[pl.ds(p0, TM // 2), :] = xn
        buf[...] = xn

    def kt_stage(buf):
        kT = _dot_nt(_up(wkT_v[...]), _up(buf[...]))
        pkT = _phi(kT)
        zs = pkT[:, 0:128]
        for c in range(1, TM // 128):
            zs = zs + pkT[:, c * 128:(c + 1) * 128]
        z_acc[0:D, :] += zs
        return _pk(pkT.astype(bf16))

    def v_stage(buf):
        return _pk(_dot(_up(buf[...]), _up(wvp_v[...])).astype(bf16))

    def kv_stage(pkT_p, v_p):
        for j in range(NL):
            a, b = ROWS[j]
            kv_acc[a:b, j * 128:(j + 1) * 128] += _dot(_up(pkT_p[a // 2:b // 2, :]),
                                                       _up(v_p[:, j * 128:(j + 1) * 128]))

    x_copy(0).wait()
    ln_tile(0, xa_v)
    x_copy(1).wait()
    ln_tile(1, xb_v)
    for i, (s, e) in enumerate(VCH):
        c_wv[i].wait()
        va_v[:, s:e] = _pk(_dot(_up(xa_v[...]), wv_v[:, s:e]).astype(bf16))
        if i == len(VCH) - 1:
            x_copy(2).wait()
            ln_tile(2, xc_v)
            wvp_v[...] = _pk(wv_v[...])
        vb_v[:, s:e] = _pk(_dot(_up(xb_v[...]), wv_v[:, s:e]).astype(bf16))
    vx_v[:, 0:V2] = _pk(_dot(_up(xc_v[...]), _up(wvp_v[:, 0:V2])).astype(bf16))
    c_wk.wait()
    wkT_v[...] = _pk(wk_v[...].T)
    vx_v[:, V2:D] = _pk(_dot(_up(xc_v[...]), _up(wvp_v[:, V2:D])).astype(bf16))
    pk0 = kt_stage(xa_v)
    pk_v[...] = kt_stage(xb_v)
    xa_v[...] = xc_v[...]
    kv_stage(pk0, va_v[...])

    def phase0_body(i, last):
        kv_stage(pk_v[...], vb_v[...])
        ln_tile(2 * i + 1, xb_v)
        pkx = kt_stage(xa_v)
        pky = kt_stage(xb_v)
        kv_stage(pkx, vx_v[...])
        if last:
            kv_stage(pky, v_stage(xb_v))
        else:
            ln_tile(2 * i + 2, xa_v)
            pk_v[...] = pky
            vb_v[...] = v_stage(xb_v)
            vx_v[...] = v_stage(xa_v)

    def phase0(i, carry):
        x_copy(2 * i + 1).wait()
        x_copy(2 * i + 2).wait()
        phase0_body(i, False)
        return carry

    lax.fori_loop(1, NT // 2 - 1, phase0, 0)
    x_copy(NT - 1).wait()
    c_wo.wait()
    c_wq.wait()
    for n in range(NL):
        wqT32[n, 0:D, :] = wq_v[n * 128:(n + 1) * 128, :].astype(f32).T
    for d in range(DH):
        for n in range(NL):
            wqTp_v[d * H // 2:(d + 1) * H // 2, n * 128:(n + 1) * 128] = _pk(
                wqT32[n, pl.ds(d, H, stride=DH), :].astype(bf16))
    phase0_body(NT // 2 - 1, True)

    def q_rows(prows):
        return _phi(_dot_nt(_up(xn_v[prows, :]), _up(wqTp_v[...])))

    def den_stage(pq):
        t = pq * zrow_v[...]
        s = t[:, 0:128]
        for j in range(1, NL):
            s = s + t[:, j * 128:(j + 1) * 128]
        s = s + pltpu.roll(s, 64, 1)
        s = s + pltpu.roll(s, 32, 1)
        r = 1.0 / (s + 1e-6)
        return jnp.concatenate([pq[:, j * 128:(j + 1) * 128] * r for j in range(NL)], axis=1).astype(bf16)

    def attn_rows(rows, hn_prows, pqn):
        attn = _dot(pqn, _up(m_v[...]))
        h = x_v[rows, :].astype(f32) + attn
        h_v[rows, :] = h
        hn_v[hn_prows, :] = _pk(_ln(h).astype(bf16))

    HM = TM // 2
    pq_top = q_rows(pl.ds(0, HM // 2))
    for j in range(NL):
        a, b = ROWS[j]
        d_idx = a + lax.broadcasted_iota(jnp.int32, (b - a, 128), 0)
        e_idx = j * 128 + lax.broadcasted_iota(jnp.int32, (b - a, 128), 1)
        same = _head(d_idx) == _head(e_idx)
        kvj = jnp.where(same, kv_acc[a:b, j * 128:(j + 1) * 128], 0.0).astype(bf16)
        mj = _dot(kvj, wo_v[j * 128:(j + 1) * 128, :])
        for n in range(NL):
            m_acc[n, a:b, :] += mj[:, n * 128:(n + 1) * 128]
    pq_bot = q_rows(pl.ds(HM // 2, HM // 2))
    for d in range(DH):
        for n in range(NL):
            m_v[d * H // 2:(d + 1) * H // 2, n * 128:(n + 1) * 128] = _pk(
                m_acc[n, pl.ds(d, H, stride=DH), :].astype(bf16))
        zp_v[d * H:(d + 1) * H, :] = z_acc[pl.ds(d, H, stride=DH), :]
    zrow_v[...] = jnp.sum(zp_v[...].T, axis=0, keepdims=True)

    attn_rows(pl.ds(0, HM), pl.ds(0, HM // 2), den_stage(pq_top))
    attn_rows(pl.ds(HM, HM), pl.ds(HM // 2, HM // 2), den_stage(pq_bot))
    c_wg.wait()
    c_wu.wait()
    c_wd.wait()

    def phase1(t, carry):
        r0 = pl.multiple_of(t * TM, TM)
        r1 = pl.multiple_of(t * TM + TM, TM)
        p1 = pl.multiple_of(t * (TM // 2) + TM // 2, TM // 2)
        hn = _up(hn_v[...])
        gate = _dot(hn, wg_v[...])
        pq = q_rows(pl.ds(p1, TM // 2))
        up = _dot(hn, wu_v[...])
        pqn = den_stage(pq)
        hh = (jnp.maximum(gate, 0.0) * up).astype(bf16)
        attn_rows(pl.ds(r1, TM), pl.ds(0, TM // 2), pqn)
        out = h_v[pl.ds(r0, TM), :] + _dot(hh, wd_v[...])
        out_v[pl.ds(r0, TM), :] = out.astype(bf16)
        o_copy(t).start()
        return carry

    lax.fori_loop(0, NT - 1, phase1, 0)
    hn = _up(hn_v[...])
    gate = _dot(hn, wg_v[...])
    up = _dot(hn, wu_v[...])
    hh = (jnp.maximum(gate, 0.0) * up).astype(bf16)
    base = (NT - 1) * TM
    last_copies = []
    for ci, (a, b) in enumerate(LAST_SPLIT):
        out = h_v[base + a:base + b, :] + _dot(hh[a:b, :], wd_v[...])
        out_v[base + a:base + b, :] = out.astype(bf16)
        cp = pltpu.make_async_copy(out_v.at[pl.ds(base + a, b - a)], out_hbm.at[pl.ds(base + a, b - a)],
                                   sem_o.at[NT - 1 + ci])
        cp.start()
        last_copies.append(cp)
    for t in range(NT - 1):
        o_copy(t).wait()
    for cp in last_copies:
        cp.wait()


@jax.jit
def pallas_sequential_preLN__linear_attn_block__glu_gated_reglu__prompt_kernel(
    A_x, A_wqkv, A_wo, B_x, B_W_gate, B_W_up, B_W_down):
    x2 = A_x.reshape(S, D)
    any_spec = pl.BlockSpec(memory_space=pl.ANY)
    out = pl.pallas_call(
        _kernel,
        out_shape=jax.ShapeDtypeStruct((S, D), bf16),
        in_specs=[any_spec] * 6,
        out_specs=any_spec,
        scratch_shapes=[
            pltpu.VMEM((S, D), bf16),
            pltpu.VMEM((S // 2, D), u32),
            pltpu.VMEM((S, D), bf16),
            pltpu.VMEM((D, D), bf16),
            pltpu.VMEM((D, D), bf16),
            pltpu.VMEM((D, D), bf16),
            pltpu.VMEM((D // 2, D), u32),
            pltpu.VMEM((D, D), bf16),
            pltpu.VMEM((D, F), bf16),
            pltpu.VMEM((D, F), bf16),
            pltpu.VMEM((F, D), bf16),
            pltpu.VMEM((D, D), f32),
            pltpu.VMEM((DP, 128), f32),
            pltpu.VMEM((NL, DP, 128), f32),
            pltpu.VMEM((D // 2, D), u32),
            pltpu.VMEM((NL, DP, 128), f32),
            pltpu.VMEM((D // 2, D), u32),
            pltpu.VMEM((D, 128), f32),
            pltpu.VMEM((TM // 2, D), u32),
            pltpu.VMEM((TM // 2, D), u32),
            pltpu.VMEM((S, D), f32),
            pltpu.VMEM((TM // 2, D), u32),
            pltpu.VMEM((TM // 2, D), u32),
            pltpu.VMEM((TM // 2, D), u32),
            pltpu.VMEM((D // 2, TM), u32),
            pltpu.VMEM((D // 2, D), u32),
            pltpu.VMEM((TM // 2, D), u32),
            pltpu.VMEM((TM // 2, D), u32),
            pltpu.VMEM((1, D), f32),
            pltpu.SemaphoreType.DMA((NT,)),
            pltpu.SemaphoreType.DMA((NT + len(LAST_SPLIT) - 1,)),
            pltpu.SemaphoreType.DMA((7 + len(VCH),)),
        ],
        compiler_params=pltpu.CompilerParams(vmem_limit_bytes=100 * 1024 * 1024),
    )(x2, A_wqkv, A_wo, B_W_gate, B_W_up, B_W_down)
    return out.reshape(A_x.shape)
```
